```python
import jax
import jax.numpy as jnp

def _softmax(x, axis=-1):
    return jax.nn.softmax(x, axis=axis)
def _gelu(x):
    return jax.nn.gelu(x, approximate=True)
def _silu(x):
    return jax.nn.silu(x)
def _sigmoid(x):
    return jax.nn.sigmoid(x)
def _layernorm(x, axis=-1, eps=1e-5):
    m = jnp.mean(x, axis=axis, keepdims=True)
    v = jnp.var(x, axis=axis, keepdims=True)
    return (x - m) / jnp.sqrt(v + eps)
def _scatter_add(tgt, idx, src, axis=0):
    return tgt.at[idx].add(src)
def _segment_sum(src, seg, n):
    return jax.ops.segment_sum(src, seg, n)
class _Rng:
    def __init__(self, key):
        self._k = key
    def _next(self):
        self._k, sub = jax.random.split(self._k)
        return sub
    def normal(self, shape):
        return jax.random.normal(self._next(), shape, dtype=jnp.bfloat16)
    def randint(self, lo, hi, shape):
        return jax.random.randint(self._next(), shape, lo, hi, dtype=jnp.int32)
    def uniform(self, shape, lo=0.0, hi=1.0):
        return jax.random.uniform(self._next(), shape, jnp.bfloat16, lo, hi)
    def permutation(self, n):
        return jax.random.permutation(self._next(), n)


kernel_name = 'standalone__cross_network_dcn_v2__recsys'

def setup_inputs():
    _rng = _Rng(jax.random.key(int.from_bytes(__import__("os").urandom(4), "little")))
    _w = (lambda a: (lambda t: t.astype(jnp.bfloat16) if jnp.issubdtype(t.dtype, jnp.floating) else t)(jnp.asarray(a)))
    B, F, D, L = 16384, 100, 16, 3
    Din = min(F * D, 512)
    R = max(Din // 4, 2)
    sc = Din ** -0.5
    return {
        "x0": _w((lambda *s: _rng.normal(s) * 0.05)(B, Din)),
        "U":  _w((lambda *s: _rng.normal(s) * 0.05)(L, Din, R) * sc),
        "V":  _w((lambda *s: _rng.normal(s) * 0.05)(L, R, Din) * sc),
        "bs": _w((lambda *s: _rng.normal(s) * 0.05)(L, Din)),
    }

def reference(x0, U, V, bs):
    x = x0
    for l in range(U.shape[0]):
        h = jnp.einsum('rd,bd->br', V[l], x)
        h = jnp.einsum('dr,br->bd', U[l], h)
        x = x0 * (h + bs[l]) + x
    return x
```

```python
import jax
import jax.numpy as jnp
from jax import lax
import jax.experimental.pallas as pl
import jax.experimental.pallas.tpu as pltpu

_NT = (((1,), (1,)), ((), ()))

_PRO = (256, 512, 1280, 2048)
_BODY = 4096
_OC = 256
_SUB = 256
_AHEAD = 2


def _cross_tile(x0b, u_ref, v_ref, b_ref):
    x0 = x0b.astype(jnp.float32)
    x = x0
    xb = x0b
    for l in range(u_ref.shape[0]):
        h = lax.dot_general(xb, v_ref[l], _NT, preferred_element_type=jnp.float32)
        g = lax.dot_general(h.astype(u_ref.dtype), u_ref[l], _NT,
                            preferred_element_type=jnp.float32)
        x = x0 * (g + b_ref[pl.ds(l, 1), :].astype(jnp.float32)) + x
        xb = x.astype(x0b.dtype)
    return xb


def _kernel(x_hbm, u_hbm, v_hbm, b_hbm, o_hbm,
            xbuf, obuf, u_ref, v_ref, b_ref, psem, isem, posem, osem, wsem):
    batch = x_hbm.shape[0]
    n_pro = len(_PRO)
    pro_rows = sum(_PRO)
    n_iter = (batch - pro_rows) // _BODY
    n_oc = _BODY // _OC
    starts = [sum(_PRO[:c]) for c in range(n_pro + 1)]

    def pro_in(c):
        r = pl.ds(starts[c], _PRO[c])
        return pltpu.make_async_copy(x_hbm.at[r], xbuf.at[r], psem.at[c])

    def loop_in(i):
        r = pl.ds(pl.multiple_of(pro_rows + i * _BODY, _SUB), _BODY)
        return pltpu.make_async_copy(x_hbm.at[r], xbuf.at[r], isem.at[i])

    def any_in(k):
        return pro_in(k) if k < n_pro else loop_in(k - n_pro)

    def pro_out():
        r = pl.ds(0, pro_rows)
        return pltpu.make_async_copy(obuf.at[r], o_hbm.at[r], posem.at[0])

    def loop_out(j):
        r = pl.ds(pl.multiple_of(pro_rows + j * _OC, _OC), _OC)
        return pltpu.make_async_copy(obuf.at[r], o_hbm.at[r], osem.at[j])

    weights = [
        pltpu.make_async_copy(v_hbm, v_ref, wsem.at[0]),
        pltpu.make_async_copy(u_hbm, u_ref, wsem.at[1]),
        pltpu.make_async_copy(b_hbm, b_ref, wsem.at[2]),
    ]
    any_in(0).start()
    for w in weights:
        w.start()
    for k in range(1, _AHEAD):
        any_in(k).start()
    for w in weights:
        w.wait()

    for c in range(n_pro):
        any_in(c).wait()
        if c + _AHEAD < n_pro + n_iter:
            any_in(c + _AHEAD).start()
        for pos in range(starts[c], starts[c + 1], _SUB):
            r = pl.ds(pos, _SUB)
            obuf[r, :] = _cross_tile(xbuf[r, :], u_ref, v_ref, b_ref)
    pro_out().start()

    def body(i, carry):
        loop_in(i).wait()

        @pl.when(i + _AHEAD < n_iter)
        def _():
            loop_in(i + _AHEAD).start()

        for g in range(n_oc):
            for s in range(_OC // _SUB):
                r = pl.ds(pl.multiple_of(pro_rows + i * _BODY + g * _OC + s * _SUB, _SUB), _SUB)
                obuf[r, :] = _cross_tile(xbuf[r, :], u_ref, v_ref, b_ref)
            loop_out(i * n_oc + g).start()
        return carry

    lax.fori_loop(0, n_iter, body, 0)
    pro_out().wait()
    for j in range(n_iter * n_oc):
        loop_out(j).wait()


@jax.jit
def pallas_standalone__cross_network_dcn_v2__recsys_kernel(
    x0: jax.Array,
    U: jax.Array,
    V: jax.Array,
    bs: jax.Array,
):
    batch = x0.shape[0]
    n_iter = (batch - sum(_PRO)) // _BODY
    assert sum(_PRO) + n_iter * _BODY == batch
    return pl.pallas_call(
        _kernel,
        in_specs=[pl.BlockSpec(memory_space=pl.ANY)] * 4,
        out_specs=pl.BlockSpec(memory_space=pl.ANY),
        out_shape=jax.ShapeDtypeStruct(x0.shape, x0.dtype),
        scratch_shapes=[
            pltpu.VMEM(x0.shape, x0.dtype),
            pltpu.VMEM(x0.shape, x0.dtype),
            pltpu.VMEM(U.shape, U.dtype),
            pltpu.VMEM(V.shape, V.dtype),
            pltpu.VMEM(bs.shape, bs.dtype),
            pltpu.SemaphoreType.DMA((len(_PRO),)),
            pltpu.SemaphoreType.DMA((n_iter,)),
            pltpu.SemaphoreType.DMA((1,)),
            pltpu.SemaphoreType.DMA((n_iter * (_BODY // _OC),)),
            pltpu.SemaphoreType.DMA((3,)),
        ],
        compiler_params=pltpu.CompilerParams(vmem_limit_bytes=64 << 20),
    )(x0, U, V, bs)
```

```python
import jax
import jax.numpy as jnp
from jax import lax
import jax.experimental.pallas as pl
import jax.experimental.pallas.tpu as pltpu

_NT = (((1,), (1,)), ((), ()))
_NN = (((1,), (0,)), ((), ()))

_TILE = 256
_RAMP = (256, 256, 256, 512, 1024, 1792)
_BODY = 6144
_TAIL = (64, 64, 64, 64)
_NSEM = 6
_TRANSPOSE_IN = 1


def _kernel(x_hbm, u_hbm, v_hbm, b_hbm, o_hbm,
            xbuf, obuf, u_ref, v_ref, b_ref, ut_ref, vt_ref, sem):
    n_layers = u_hbm.shape[0]
    ramp_rows = sum(_RAMP)
    n_iter = (x_hbm.shape[0] - ramp_rows) // _BODY
    ramp_start = [sum(_RAMP[:c]) for c in range(len(_RAMP))]
    first_body = n_layers + len(_RAMP) - 1
    n_stages = first_body + n_iter
    assert n_stages - _NSEM <= first_body
    out_sem = n_stages % _NSEM

    def low_rank(xb, l, transposed):
        if transposed:
            h = lax.dot_general(xb, vt_ref[l], _NN, preferred_element_type=jnp.float32)
            return lax.dot_general(h.astype(xb.dtype), ut_ref[l], _NN,
                                   preferred_element_type=jnp.float32)
        h = lax.dot_general(xb, v_ref[l], _NT, preferred_element_type=jnp.float32)
        return lax.dot_general(h.astype(xb.dtype), u_ref[l], _NT,
                               preferred_element_type=jnp.float32)

    def cross(x0b, xb, g, l):
        bias = b_ref[pl.ds(l, 1), :].astype(jnp.float32)
        return (x0b.astype(jnp.float32) * (g + bias)
                + xb.astype(jnp.float32)).astype(xb.dtype)

    def layers(x0b, xb, ls, transposed):
        for l in ls:
            xb = cross(x0b, xb, low_rank(xb, l, transposed), l)
        return xb

    def x_in(start, rows, s):
        r = pl.ds(start, rows)
        return pltpu.make_async_copy(x_hbm.at[r], xbuf.at[r], sem.at[s])

    def x_out(start, rows):
        r = pl.ds(start, rows)
        return pltpu.make_async_copy(obuf.at[r], o_hbm.at[r], sem.at[out_sem])

    def stage(k):
        s = k % _NSEM
        if k < n_layers:
            v = pltpu.make_async_copy(v_hbm.at[k], v_ref.at[k], sem.at[s])
            u = pltpu.make_async_copy(u_hbm.at[k], u_ref.at[k], sem.at[s])
            if k > 0:
                return [v, u]
            return [v, x_in(0, _RAMP[0], s), u,
                    pltpu.make_async_copy(b_hbm, b_ref, sem.at[s])]
        if k < first_body:
            c = k - n_layers + 1
            return [x_in(ramp_start[c], _RAMP[c], s)]
        return [x_in(ramp_rows + (k - first_body) * _BODY, _BODY, s)]

    def finish_stage(k):
        for copy in stage(k):
            copy.wait()
        if k + _NSEM < n_stages:
            for copy in stage(k + _NSEM):
                copy.start()

    def ramp():
        for k in range(_NSEM):
            for copy in stage(k):
                copy.start()
        rows = pl.ds(0, _RAMP[0])
        for l in range(n_layers):
            finish_stage(l)
            x0b = xbuf[rows, :]
            xb = x0b if l == 0 else obuf[rows, :]
            obuf[rows, :] = layers(x0b, xb, [l], False)
        for c in range(1, len(_RAMP)):
            finish_stage(n_layers - 1 + c)
            if c == _TRANSPOSE_IN:
                for l in range(n_layers):
                    vt_ref[l] = v_ref[l].T
                    ut_ref[l] = u_ref[l].T
            for start in range(ramp_start[c], ramp_start[c] + _RAMP[c], _TILE):
                rows = pl.ds(start, _TILE)
                x0b = xbuf[rows, :]
                obuf[rows, :] = layers(x0b, x0b, range(n_layers), c > _TRANSPOSE_IN)
        x_out(0, ramp_rows).start(priority=1)

    def body(i):
        base = ramp_rows + i * _BODY
        x_in(pl.multiple_of(base, _TILE), _BODY, (first_body + i) % _NSEM).wait()
        for pos in range(0, _BODY - _TILE, _TILE):
            start = pl.multiple_of(base + pos, _TILE)
            x0b = xbuf[pl.ds(start, _TILE), :]
            obuf[pl.ds(start, _TILE), :] = layers(x0b, x0b, range(n_layers), True)
            x_out(start, _TILE).start(priority=1)
        pos = _BODY - _TILE
        x0b = xbuf[pl.ds(pl.multiple_of(base + pos, _TILE), _TILE), :]
        xb = layers(x0b, x0b, range(n_layers - 1), True)
        g = low_rank(xb, n_layers - 1, True)
        p = 0
        for n in _TAIL:
            start = pl.multiple_of(base + pos + p, min(_TAIL))
            obuf[pl.ds(start, n), :] = cross(
                x0b[p:p + n], xb[p:p + n], g[p:p + n], n_layers - 1)
            x_out(start, n).start(priority=1)
            p += n

    def step(i, carry):
        pl.when(i == 0)(ramp)
        pl.when(i > 0)(lambda: body(i - 1))
        return carry

    lax.fori_loop(0, n_iter + 1, step, 0)
    pltpu.make_async_copy(obuf, o_hbm, sem.at[out_sem]).wait()


@jax.jit
def pallas_standalone__cross_network_dcn_v2__recsys_kernel(
    x0: jax.Array,
    U: jax.Array,
    V: jax.Array,
    bs: jax.Array,
):
    batch = x0.shape[0]
    assert batch > sum(_RAMP) and (batch - sum(_RAMP)) % _BODY == 0
    return pl.pallas_call(
        _kernel,
        in_specs=[pl.BlockSpec(memory_space=pl.ANY)] * 4,
        out_specs=pl.BlockSpec(memory_space=pl.ANY),
        out_shape=jax.ShapeDtypeStruct(x0.shape, x0.dtype),
        scratch_shapes=[
            pltpu.VMEM(x0.shape, x0.dtype),
            pltpu.VMEM(x0.shape, x0.dtype),
            pltpu.VMEM(U.shape, U.dtype),
            pltpu.VMEM(V.shape, V.dtype),
            pltpu.VMEM(bs.shape, bs.dtype),
            pltpu.VMEM(V.shape, U.dtype),
            pltpu.VMEM(U.shape, V.dtype),
            pltpu.SemaphoreType.DMA((_NSEM,)),
        ],
        compiler_params=pltpu.CompilerParams(
            vmem_limit_bytes=64 << 20,
            flags={"XLA_TPU_RESCHEDULE_DMA_DONES": True},
        ),
    )(x0, U, V, bs)
```

```python
import jax
import jax.numpy as jnp
from jax import lax
import jax.experimental.pallas as pl
import jax.experimental.pallas.tpu as pltpu

_NT = (((1,), (1,)), ((), ()))
_NN = (((1,), (0,)), ((), ()))

_TILE = 256
_RAMP = (256, 256, 256, 512, 1024, 1792)
_BODY = 6144
_TAIL = (64, 64, 64, 64)
_NSEM = 3
_TRANSPOSE_IN = 1


def _kernel(x_hbm, u_hbm, v_hbm, b_hbm, o_hbm,
            xbuf, obuf, u_ref, v_ref, b_ref, ut_ref, vt_ref, sem):
    n_layers = u_hbm.shape[0]
    ramp_rows = sum(_RAMP)
    n_iter = (x_hbm.shape[0] - ramp_rows) // _BODY
    ramp_start = [sum(_RAMP[:c]) for c in range(len(_RAMP))]
    first_body = n_layers + len(_RAMP) - 1
    n_stages = first_body + n_iter
    assert n_iter < _NSEM
    out_sem = n_stages % _NSEM

    def low_rank(xb, l, transposed):
        if transposed:
            h = lax.dot_general(xb, vt_ref[l], _NN, preferred_element_type=jnp.float32)
            return lax.dot_general(h.astype(xb.dtype), ut_ref[l], _NN,
                                   preferred_element_type=jnp.float32)
        h = lax.dot_general(xb, v_ref[l], _NT, preferred_element_type=jnp.float32)
        return lax.dot_general(h.astype(xb.dtype), u_ref[l], _NT,
                               preferred_element_type=jnp.float32)

    def cross(x0b, xb, g, l):
        bias = b_ref[pl.ds(l, 1), :].astype(jnp.float32)
        return (x0b.astype(jnp.float32) * (g + bias)
                + xb.astype(jnp.float32)).astype(xb.dtype)

    def layers(x0b, xb, ls, transposed):
        for l in ls:
            xb = cross(x0b, xb, low_rank(xb, l, transposed), l)
        return xb

    def x_in(start, rows, s):
        r = pl.ds(start, rows)
        return pltpu.make_async_copy(x_hbm.at[r], xbuf.at[r], sem.at[s])

    def x_out(start, rows):
        r = pl.ds(start, rows)
        return pltpu.make_async_copy(obuf.at[r], o_hbm.at[r], sem.at[out_sem])

    def stage(k):
        s = k % _NSEM
        if k < n_layers:
            v = pltpu.make_async_copy(v_hbm.at[k], v_ref.at[k], sem.at[s])
            u = pltpu.make_async_copy(u_hbm.at[k], u_ref.at[k], sem.at[s])
            if k > 0:
                return [v, u]
            return [v, x_in(0, _RAMP[0], s), u,
                    pltpu.make_async_copy(b_hbm, b_ref, sem.at[s])]
        if k < first_body:
            c = k - n_layers + 1
            return [x_in(ramp_start[c], _RAMP[c], s)]
        return [x_in(ramp_rows + (k - first_body) * _BODY, _BODY, s)]

    def finish_stage(k):
        for copy in stage(k):
            copy.wait()
        if k + _NSEM < n_stages:
            for copy in stage(k + _NSEM):
                copy.start()

    def ramp():
        for k in range(_NSEM):
            for copy in stage(k):
                copy.start()
        rows = pl.ds(0, _RAMP[0])
        finish_stage(0)
        x0b = xbuf[rows, :]
        xb = layers(x0b, x0b, [0], False)
        for l in range(1, n_layers):
            finish_stage(l)
            xb = layers(x0b, xb, [l], False)
        obuf[rows, :] = xb
        for c in range(1, len(_RAMP)):
            finish_stage(n_layers - 1 + c)
            if c == _TRANSPOSE_IN:
                for l in range(n_layers):
                    vt_ref[l] = v_ref[l].T
                    ut_ref[l] = u_ref[l].T
            for start in range(ramp_start[c], ramp_start[c] + _RAMP[c], _TILE):
                rows = pl.ds(start, _TILE)
                x0b = xbuf[rows, :]
                obuf[rows, :] = layers(x0b, x0b, range(n_layers), c > _TRANSPOSE_IN)
        x_out(0, ramp_rows).start(priority=1)

    def body(i):
        base = ramp_rows + i * _BODY
        x_in(pl.multiple_of(base, _TILE), _BODY, (first_body + i) % _NSEM).wait()
        for pos in range(0, _BODY - _TILE, _TILE):
            start = pl.multiple_of(base + pos, _TILE)
            x0b = xbuf[pl.ds(start, _TILE), :]
            obuf[pl.ds(start, _TILE), :] = layers(x0b, x0b, range(n_layers), True)
            x_out(start, _TILE).start(priority=1)
        pos = _BODY - _TILE
        x0b = xbuf[pl.ds(pl.multiple_of(base + pos, _TILE), _TILE), :]
        xb = layers(x0b, x0b, range(n_layers - 1), True)
        g = low_rank(xb, n_layers - 1, True)
        p = 0
        for n in _TAIL:
            start = pl.multiple_of(base + pos + p, min(_TAIL))
            obuf[pl.ds(start, n), :] = cross(
                x0b[p:p + n], xb[p:p + n], g[p:p + n], n_layers - 1)
            x_out(start, n).start(priority=1)
            p += n

    def step(i, carry):
        pl.when(i == 0)(ramp)
        pl.when(i > 0)(lambda: body(i - 1))
        return carry

    lax.fori_loop(0, n_iter + 1, step, 0)
    pltpu.make_async_copy(obuf, o_hbm, sem.at[out_sem]).wait()


@jax.jit
def pallas_standalone__cross_network_dcn_v2__recsys_kernel(
    x0: jax.Array,
    U: jax.Array,
    V: jax.Array,
    bs: jax.Array,
):
    batch = x0.shape[0]
    assert batch > sum(_RAMP) and (batch - sum(_RAMP)) % _BODY == 0
    return pl.pallas_call(
        _kernel,
        in_specs=[pl.BlockSpec(memory_space=pl.ANY)] * 4,
        out_specs=pl.BlockSpec(memory_space=pl.ANY),
        out_shape=jax.ShapeDtypeStruct(x0.shape, x0.dtype),
        scratch_shapes=[
            pltpu.VMEM(x0.shape, x0.dtype),
            pltpu.VMEM(x0.shape, x0.dtype),
            pltpu.VMEM(U.shape, U.dtype),
            pltpu.VMEM(V.shape, V.dtype),
            pltpu.VMEM(bs.shape, bs.dtype),
            pltpu.VMEM(V.shape, U.dtype),
            pltpu.VMEM(U.shape, V.dtype),
            pltpu.SemaphoreType.DMA((_NSEM,)),
        ],
        compiler_params=pltpu.CompilerParams(
            vmem_limit_bytes=64 << 20,
            flags={"XLA_TPU_RESCHEDULE_DMA_DONES": True},
        ),
    )(x0, U, V, bs)
```

```python
import jax
import jax.numpy as jnp
from jax import lax
import jax.experimental.pallas as pl
import jax.experimental.pallas.tpu as pltpu

_NT = (((1,), (1,)), ((), ()))
_NN = (((1,), (0,)), ((), ()))

_TILE = 256
_RAMP = (256, 256, 256, 512, 1024, 1792)
_BODY = 6144
_TAIL = (64, 64, 64, 64)
_NSEM = 3
_TRANSPOSE_IN = 1


def _kernel(x_hbm, u_hbm, v_hbm, b_hbm, o_hbm,
            xbuf, obuf, xv_buf, hu_buf, b_ref, ut_ref, vt_ref, sem):
    n_layers, dim, rank = u_hbm.shape
    first = _RAMP[0]
    ramp_rows = sum(_RAMP)
    n_iter = (x_hbm.shape[0] - ramp_rows) // _BODY
    ramp_start = [sum(_RAMP[:c]) for c in range(len(_RAMP))]
    first_body = n_layers + len(_RAMP) - 1
    n_stages = first_body + n_iter
    assert n_iter < _NSEM
    out_sem = n_stages % _NSEM

    head = pl.ds(0, first)

    def v_rows(l):
        return pl.ds(first + l * rank, rank)

    def u_rows(l):
        return pl.ds(first + l * dim, dim)

    def dot(a, b, dims):
        return lax.dot_general(a, b, dims, preferred_element_type=jnp.float32)

    def low_rank(xb, l, transposed):
        if transposed:
            return dot(dot(xb, vt_ref[l], _NN).astype(xb.dtype), ut_ref[l], _NN)
        h = dot(xb, xv_buf[v_rows(l), :], _NT).astype(xb.dtype)
        return dot(h, hu_buf[u_rows(l), :], _NT)

    def cross(x0b, xb, g, l):
        bias = b_ref[pl.ds(l, 1), :].astype(jnp.float32)
        return (x0b.astype(jnp.float32) * (g + bias)
                + xb.astype(jnp.float32)).astype(xb.dtype)

    def layers(x0b, count, transposed):
        xb = x0b
        for l in range(count):
            xb = cross(x0b, xb, low_rank(xb, l, transposed), l)
        return xb

    def x_in(start, rows, s):
        r = pl.ds(start, rows)
        return pltpu.make_async_copy(x_hbm.at[r], xbuf.at[r], sem.at[s])

    def x_out(start, rows):
        r = pl.ds(start, rows)
        return pltpu.make_async_copy(obuf.at[r], o_hbm.at[r], sem.at[out_sem])

    def stage(k):
        s = k % _NSEM
        if k < n_layers:
            v = pltpu.make_async_copy(v_hbm.at[k], xv_buf.at[v_rows(k)], sem.at[s])
            u = pltpu.make_async_copy(u_hbm.at[k], hu_buf.at[u_rows(k)], sem.at[s])
            if k > 0:
                return [v, u]
            return [v,
                    pltpu.make_async_copy(x_hbm.at[head], xv_buf.at[head], sem.at[s]),
                    u,
                    pltpu.make_async_copy(b_hbm, b_ref, sem.at[s])]
        if k < first_body:
            c = k - n_layers + 1
            return [x_in(ramp_start[c], _RAMP[c], s)]
        return [x_in(ramp_rows + (k - first_body) * _BODY, _BODY, s)]

    def finish_stage(k):
        for copy in stage(k):
            copy.wait()
        if k + _NSEM < n_stages:
            for copy in stage(k + _NSEM):
                copy.start()

    def ramp():
        for k in range(_NSEM):
            for copy in stage(k):
                copy.start()
        finish_stage(0)
        xb = xv_buf[head, :]
        for l in range(n_layers):
            if l > 0:
                finish_stage(l)
            hu_buf[head, :] = dot(xb, xv_buf[v_rows(l), :], _NT).astype(xb.dtype)
            h = hu_buf[head, :]
            x0b = xv_buf[head, :]
            xb = cross(x0b, xb, dot(h, hu_buf[u_rows(l), :], _NT), l)
        obuf[head, :] = xb
        for c in range(1, len(_RAMP)):
            finish_stage(n_layers - 1 + c)
            if c == _TRANSPOSE_IN:
                for l in range(n_layers):
                    vt_ref[l] = xv_buf[v_rows(l), :].T
                    ut_ref[l] = hu_buf[u_rows(l), :].T
            for start in range(ramp_start[c], ramp_start[c] + _RAMP[c], _TILE):
                rows = pl.ds(start, _TILE)
                obuf[rows, :] = layers(xbuf[rows, :], n_layers, c > _TRANSPOSE_IN)
        x_out(0, ramp_rows).start(priority=1)

    def body(i):
        base = ramp_rows + i * _BODY
        x_in(pl.multiple_of(base, _TILE), _BODY, (first_body + i) % _NSEM).wait()
        for pos in range(0, _BODY - _TILE, _TILE):
            start = pl.multiple_of(base + pos, _TILE)
            rows = pl.ds(start, _TILE)
            obuf[rows, :] = layers(xbuf[rows, :], n_layers, True)
            x_out(start, _TILE).start(priority=1)
        pos = _BODY - _TILE
        x0b = xbuf[pl.ds(pl.multiple_of(base + pos, _TILE), _TILE), :]
        xb = layers(x0b, n_layers - 1, True)
        g = low_rank(xb, n_layers - 1, True)
        p = 0
        for n in _TAIL:
            start = pl.multiple_of(base + pos + p, min(_TAIL))
            obuf[pl.ds(start, n), :] = cross(
                x0b[p:p + n], xb[p:p + n], g[p:p + n], n_layers - 1)
            x_out(start, n).start(priority=1)
            p += n

    def step(i, carry):
        pl.when(i == 0)(ramp)
        pl.when(i > 0)(lambda: body(i - 1))
        return carry

    lax.fori_loop(0, n_iter + 1, step, 0)
    pltpu.make_async_copy(o_hbm, o_hbm, sem.at[out_sem]).wait()


@jax.jit
def pallas_standalone__cross_network_dcn_v2__recsys_kernel(
    x0: jax.Array,
    U: jax.Array,
    V: jax.Array,
    bs: jax.Array,
):
    batch, dim = x0.shape
    n_layers, _, rank = U.shape
    assert batch > sum(_RAMP) and (batch - sum(_RAMP)) % _BODY == 0
    assert U.dtype == V.dtype == x0.dtype
    return pl.pallas_call(
        _kernel,
        in_specs=[pl.BlockSpec(memory_space=pl.ANY)] * 4,
        out_specs=pl.BlockSpec(memory_space=pl.ANY),
        out_shape=jax.ShapeDtypeStruct(x0.shape, x0.dtype),
        scratch_shapes=[
            pltpu.VMEM(x0.shape, x0.dtype),
            pltpu.VMEM(x0.shape, x0.dtype),
            pltpu.VMEM((_RAMP[0] + n_layers * rank, dim), x0.dtype),
            pltpu.VMEM((_RAMP[0] + n_layers * dim, rank), x0.dtype),
            pltpu.VMEM(bs.shape, bs.dtype),
            pltpu.VMEM(V.shape, U.dtype),
            pltpu.VMEM(U.shape, V.dtype),
            pltpu.SemaphoreType.DMA((_NSEM,)),
        ],
        compiler_params=pltpu.CompilerParams(
            vmem_limit_bytes=64 << 20,
            flags={"XLA_TPU_RESCHEDULE_DMA_DONES": True},
        ),
    )(x0, U, V, bs)
```
